```python
import os as _os
_os.environ.setdefault("JAX_PLATFORMS", "cpu")
import jax
import jax.numpy as jnp

def _softmax(x, axis=-1):
    return jax.nn.softmax(x, axis=axis)
def _gelu(x):
    return jax.nn.gelu(x, approximate=True)
def _silu(x):
    return jax.nn.silu(x)
def _sigmoid(x):
    return jax.nn.sigmoid(x)
def _layernorm(x, axis=-1, eps=1e-5):
    m = jnp.mean(x, axis=axis, keepdims=True)
    v = jnp.var(x, axis=axis, keepdims=True)
    return (x - m) / jnp.sqrt(v + eps)
def _scatter_add(tgt, idx, src, axis=0):
    return tgt.at[idx].add(src)
def _segment_sum(src, seg, n):
    return jax.ops.segment_sum(src, seg, n)
class _Rng:
    def __init__(self, key):
        self._k = key
    def _next(self):
        self._k, sub = jax.random.split(self._k)
        return sub
    def normal(self, shape):
        return jax.random.normal(self._next(), shape, dtype=jnp.bfloat16)
    def randint(self, lo, hi, shape):
        return jax.random.randint(self._next(), shape, lo, hi, dtype=jnp.int32)
    def uniform(self, shape, lo=0.0, hi=1.0):
        return jax.random.uniform(self._next(), shape, jnp.bfloat16, lo, hi)
    def permutation(self, n):
        return jax.random.permutation(self._next(), n)


kernel_name = 'sequential_preLN__mha_block__mixer_token_mlp__prompt'

def setup_inputs():
    _rng = _Rng(jax.random.key(int.from_bytes(__import__("os").urandom(4), "little")))
    _w = (lambda a: (lambda t: t.astype(jnp.bfloat16) if jnp.issubdtype(t.dtype, jnp.floating) else t)(jnp.asarray(a)))
    def _A_setup():
        B, S, D, H = 1, 2048, 448, 16
        return {
            "x": _w((lambda *s: _rng.normal(s) * 0.05)(B, S, D)),
            "wqkv": _w((lambda *s: _rng.normal(s) * 0.05)(D, 3 * D)),
            "wo": _w((lambda *s: _rng.normal(s) * 0.05)(D, D)),
        }
    _A_in = _A_setup()

    def _B_setup():
        B, S, D, F = 1, 2048, 448, 1792
        return {
            "x": _w((lambda *s: _rng.normal(s) * 0.05)(B, S, D)),
            "w1": _w((lambda *s: _rng.normal(s) * 0.2)(S, F) * (S ** -0.5)),
            "b1": _w((lambda *s: _rng.normal(s) * 0.2)(F) * 0.02),
            "w2": _w((lambda *s: _rng.normal(s) * 0.2)(F, S) * (F ** -0.5)),
            "b2": _w((lambda *s: _rng.normal(s) * 0.05)(S) * 0.02),
        }
    _B_in = _B_setup()

    return {
        "A_x": _A_in["x"],
        "A_wqkv": _A_in["wqkv"],
        "A_wo": _A_in["wo"],
        "B_x": _B_in["x"],
        "B_w1": _B_in["w1"],
        "B_b1": _B_in["b1"],
        "B_w2": _B_in["w2"],
        "B_b2": _B_in["b2"],
    }

def reference(A_x, A_wqkv, A_wo, B_x, B_w1, B_b1, B_w2, B_b2):
    def _A_ref(x, wqkv, wo):
        B, S, D = x.shape
        H = 16
        Dh = D // H
        qkv = (lambda x, *d: x.transpose(*d))((x @ wqkv).reshape(B, S, 3, H, Dh), 2, 0, 3, 1, 4)
        q, k, v = qkv[0], qkv[1], qkv[2]
        scores = jnp.einsum("bhqd,bhkd->bhqk", q, k) * (Dh ** -0.5)
        p = _softmax(scores, axis=-1)
        o = jnp.einsum("bhqk,bhkd->bhqd", p, v)
        return (lambda x, *d: x.transpose(*d))(o, 0, 2, 1, 3).reshape(B, S, D) @ wo

    def _B_ref(x, w1, b1, w2, b2):
        B, S, D = x.shape
        h = _layernorm(x, axis=-1)
        u = jnp.einsum("bsd,sf->bdf", h, w1) + b1
        u = _gelu(u)
        y = jnp.einsum("bdf,fs->bds", u, w2) + b2
        return (lambda x, *d: x.transpose(*d))(y, 0, 2, 1)

    x = A_x
    h = x + _A_ref(_layernorm(x, axis=-1), A_wqkv, A_wo)
    h2 = h + _B_ref(_layernorm(h, axis=-1), B_w1, B_b1, B_w2, B_b2)
    return h2
```

```python
import jax
import jax.numpy as jnp
import jax.experimental.pallas as pl
import jax.experimental.pallas.tpu as pltpu

S, D, H, DH, F = 2048, 448, 16, 28, 1792
HP = 32
EPS = 1e-5
LOG2E = 1.4426950408889634
SAFE_S2 = 40.0 ** 2
SAFE_V = 2.0 ** 60
CFG = dict(BQ=2048, BK=1024, NQ=2, TB=512, FB=896, SB=128, OB=512, R1=1, R2=8)
BF, F32, U32 = jnp.bfloat16, jnp.float32, jnp.uint32


def _pk(t):
    return pltpu.bitcast(t.astype(BF), U32)


def _un(t):
    return pltpu.bitcast(t, BF)


def _head(t, h, fill):
    r0 = h * DH - 4 * (h % 2)
    w = t[r0:r0 + HP]
    row = jax.lax.broadcasted_iota(jnp.int32, (8, t.shape[1]), 0)
    if h % 2 == 0:
        return jnp.concatenate([w[:24], jnp.where(row < 4, w[24:], fill)], 0)
    return jnp.concatenate([jnp.where(row >= 4, w[:8], fill), w[8:]], 0)


def _ln_t(t):
    m = jnp.sum(t, axis=0, keepdims=True) * (1.0 / D)
    c = t - m
    v = jnp.sum(c * c, axis=0, keepdims=True) * (1.0 / D)
    return c * jax.lax.rsqrt(v + EPS)


def _kernel(x_hbm, wqkv_hbm, wo_hbm, w1_hbm, b1_ref, w2_hbm, b2_ref, o_hbm,
            x_v, wqkv_v, wo_v, w1_v, w2_v, o_v,
            xt, wt, qt, kg, vt, ot, ht, ut, bias, stat, wot, flag, sems, osem):
    BQ, BK, NQ, TB, FB, SB = (CFG[k] for k in ("BQ", "BK", "NQ", "TB", "FB", "SB"))
    wcols = [(0, 512), (512, 896), (896, 3 * D)]
    xcols = [(0, TB), (TB, 2 * TB), (2 * TB, S)]
    pairs = [(x_hbm.at[:, a:b], x_v.at[:, a:b]) for a, b in xcols[:1]]
    pairs += [(wqkv_hbm.at[:, a:b], wqkv_v.at[:, a:b]) for a, b in wcols]
    pairs += [(x_hbm.at[:, a:b], x_v.at[:, a:b]) for a, b in xcols[1:]]
    first = [pltpu.make_async_copy(s, d, sems.at[i]) for i, (s, d) in enumerate(pairs)]
    cps = [pltpu.make_async_copy(s, d, sems.at[len(pairs) + i]) for i, (s, d) in enumerate(
        [(wo_hbm, wo_v), (w1_hbm, w1_v), (w2_hbm, w2_v)])]
    for cp in first + cps[:1]:
        cp.start()
    qscale = DH ** -0.5 * LOG2E
    row = jax.lax.broadcasted_iota(jnp.int32, (8, TB), 0)
    ones_row = jnp.where(row % 4 == 0, 1.0, 0.0).astype(F32)
    def ln_in(t, slot):
        xb = x_v[:, t].astype(F32)
        ht[:, TB * slot:TB * (slot + 1)] = _pk(_ln_t(xb))

    def proj(j, xn):
        return jnp.dot(_un(wt[j * (D // 2):(j + 1) * (D // 2), :]), xn, preferred_element_type=F32)

    def fold(rows):
        t = jnp.concatenate(rows, 0)
        r = t[:, 0:128]
        for c in range(128, TB, 128):
            r = jnp.maximum(r, t[:, c:c + 128])
        return r

    def post_q(q, t, t2):
        q = q * qscale
        n2 = []
        for h in range(H):
            qh = _head(q, h, 0.0)
            qt[h, :, t] = _pk(qh)
            n2.append(jnp.sum(qh * qh, 0, keepdims=True))
        stat[0:H] = jnp.maximum(stat[0:H], fold(n2))

    def post_k(k, t, t2):
        kp, n2 = [], []
        for h in range(H):
            kh = _head(k, h, 0.0)
            kp.append(kh)
            n2.append(jnp.sum(kh * kh, 0, keepdims=True))
        stat[H:2 * H] = jnp.maximum(stat[H:2 * H], fold(n2))
        for g in range(4):
            kg[g, t2, :] = _pk(jnp.concatenate(kp[4 * g:4 * g + 4], 0).T)

    def post_v(v, t, t2):
        va = jnp.max(jnp.abs(v).reshape(D // 8, 8, TB), axis=0)
        r = va[:, 0:128]
        for c in range(128, TB, 128):
            r = jnp.maximum(r, va[:, c:c + 128])
        stat[2 * H:2 * H + 8] = jnp.maximum(stat[2 * H:2 * H + 8], r)
        for h in range(H):
            vt[h, :, t] = _pk(_head(v, h, ones_row))

    posts = (post_q, post_k, post_v)
    stat[...] = jnp.zeros(stat.shape, F32)
    def w_transpose(j):
        a, b = wcols[j]
        wt[a // 2:b // 2, :] = _pk(wqkv_v[:, a:b].astype(F32).T)

    def first_proj(j):
        posts[j](proj(j, _un(ht[:, TB:2 * TB])), pl.ds(0, TB), pl.ds(0, TB // 2))

    bias[0:1, 0:F] = b1_ref[...].astype(F32).reshape(1, F)
    bias[1:2, :] = b2_ref[...].astype(F32).reshape(1, S)
    first[0].wait()
    ln_in(pl.ds(0, TB), 1)
    first[1].wait()
    w_transpose(0)
    first[2].wait()
    w_transpose(1)
    first_proj(0)
    first[3].wait()
    first[4].wait()
    w_transpose(2)
    first_proj(1)
    ln_in(pl.ds(TB, TB), 0)
    first_proj(2)
    first[5].wait()
    cps[0].wait()

    def p1(i, c):
        t = pl.ds(pl.multiple_of(i * TB, TB), TB)
        t2 = pl.ds(pl.multiple_of(i * (TB // 2), TB // 2), TB // 2)
        xn = _un(ht[:, 0:TB])
        for n, j in enumerate((1, 0, 2)):
            posts[j](proj(j, xn), t, t2)
            if n == 0:
                ln_in(pl.ds(pl.multiple_of(jnp.minimum(i + 1, S // TB - 1) * TB, TB), TB), 0)
        wo32 = wo_v[...].astype(F32)
        wot[...] = _pk(jnp.concatenate([_head(wo32, h, 0.0) for h in range(H)], 0).T)
        return c
    jax.lax.fori_loop(1, S // TB, p1, 0)

    smax = jnp.max(stat[...], axis=1, keepdims=True)
    bound = jnp.max(smax[0:H] * smax[H:2 * H])
    vmax = jnp.max(smax[2 * H:2 * H + 8])
    flag[0] = jnp.where((bound <= SAFE_S2) & (vmax <= SAFE_V), 1, 0)

    def masked_q(h, q0):
        qb = qt[h, :, pl.ds(q0, BQ)]
        z = jnp.zeros(qb.shape, U32)
        return _un(jnp.concatenate([jnp.where(h % 4 == j, qb, z) for j in range(4)], 0))

    def finish(h, q0, acc):
        inv = 1.0 / jnp.where(h % 2 == 0, acc[DH:DH + 1, :], acc[0:1, :])
        ot[pl.ds(pl.multiple_of(h * (HP // 2), HP // 2), HP // 2), pl.ds(q0, BQ)] = _pk(acc * inv)

    @pl.when(flag[0] == 1)
    def _():
        def body(i, c):
            @pl.when(i == 0)
            def _():
                for cp in cps[1:]:
                    cp.start()
            for j in range(NQ):
                n = i * NQ + j
                h = n // (S // BQ)
                q0 = pl.multiple_of((n % (S // BQ)) * BQ, BQ)
                rhs = masked_q(h, q0)
                acc = jnp.zeros((HP, BQ), F32)
                for k0 in range(0, S, BK):
                    s = jnp.dot(_un(kg[h // 4, k0 // 2:(k0 + BK) // 2, :]), rhs, preferred_element_type=F32)
                    p = jnp.exp2(s).astype(BF)
                    acc = acc + jnp.dot(_un(vt[h, :, k0:k0 + BK]), p, preferred_element_type=F32)
                finish(h, q0, acc)
            return c
        jax.lax.fori_loop(0, H // NQ, body, 0)

    @pl.when(flag[0] != 1)
    def _():
        for cp in cps[1:]:
            cp.start()
        def body(n, c):
            h = n // (S // BQ)
            q0 = pl.multiple_of((n % (S // BQ)) * BQ, BQ)
            rhs = masked_q(h, q0)

            def kstep(kk, carry):
                m, acc = carry
                k0 = pl.multiple_of(kk * 128, 128)
                k2 = pl.multiple_of(kk * 64, 64)
                s = jnp.dot(_un(kg[h // 4, pl.ds(k2, 64), :]), rhs, preferred_element_type=F32)
                mn = jnp.maximum(m, jnp.max(s, axis=0, keepdims=True))
                p = jnp.exp2(s - mn).astype(BF)
                acc = acc * jnp.exp2(m - mn) + jnp.dot(_un(vt[h, :, pl.ds(k0, 128)]), p, preferred_element_type=F32)
                return mn, acc
            _, acc = jax.lax.fori_loop(
                0, S // 128, kstep, (jnp.full((1, BQ), -jnp.inf, F32), jnp.zeros((HP, BQ), F32)))
            finish(h, q0, acc)
            return c
        jax.lax.fori_loop(0, H * S // BQ, body, 0)

    OB = CFG['OB']
    for t0 in range(0, S, OB):
        hb = x_v[:, t0:t0 + OB].astype(F32) + jnp.dot(_un(wot[...]), _un(ot[:, t0:t0 + OB]), preferred_element_type=F32)
        xt[:, t0:t0 + OB] = hb
        ht[:, t0:t0 + OB] = _pk(_ln_t(hb))

    cps[1].wait()

    def loop(n, body, rolled):
        if rolled:
            w = [c for c in range(1, n + 1) if n % c == 0 and c <= rolled][-1]
            def outer(i, c):
                for j in range(w):
                    body(i * w + j)
                return c
            jax.lax.fori_loop(0, n // w, outer, 0)
        else:
            for i in range(n):
                body(i)


    def mlp1(i):
        f = pl.ds(pl.multiple_of(i * FB, FB), FB)
        u = jnp.dot(_un(ht[...]), w1_v[:, f], preferred_element_type=F32) + bias[0:1, f]
        ut[:, f] = _pk(0.5 * u * (1.0 + jnp.tanh(0.7978845608028654 * (u + 0.044715 * (u * u * u)))))
    loop(F // FB, mlp1, CFG["R1"])
    cps[2].wait()

    def mlp2(i):
        t = pl.ds(pl.multiple_of(i * SB, SB), SB)
        y = jnp.dot(_un(ut[...]), w2_v[:, t], preferred_element_type=F32) + bias[1:2, t] + xt[:, t]
        o_v[:, t] = y.astype(BF)
        pltpu.make_async_copy(o_v.at[:, t], o_hbm.at[:, t], osem).start()
    loop(S // SB, mlp2, CFG["R2"])
    pltpu.make_async_copy(o_v, o_hbm, osem).wait()


@jax.jit
def pallas_sequential_preLN__mha_block__mixer_token_mlp__prompt_kernel(
    A_x, A_wqkv, A_wo, B_x, B_w1, B_b1, B_w2, B_b2,
):
    del B_x
    hbm = pl.BlockSpec(memory_space=pltpu.HBM)
    vm = pl.BlockSpec(memory_space=pltpu.VMEM)
    V = pltpu.VMEM
    out = pl.pallas_call(
        _kernel,
        out_shape=jax.ShapeDtypeStruct((D, S), BF),
        in_specs=[hbm, hbm, hbm, hbm, vm, hbm, vm],
        out_specs=hbm,
        scratch_shapes=[
            V((D, S), BF), V((D, 3 * D), BF), V((D, D), BF), V((S, F), BF), V((F, S), BF), V((D, S), BF),
            V((D, S), F32), V((3 * D // 2, D), U32), V((H, HP // 2, S), U32), V((4, S // 2, 128), U32),
            V((H, HP // 2, S), U32),
            V((H * HP // 2, S), U32), V((D // 2, S), U32), V((D // 2, F), U32), V((8, S), F32), V((2 * H + 8, 128), F32),
            V((D // 2, H * HP), U32),
            pltpu.SMEM((1,), jnp.int32), pltpu.SemaphoreType.DMA((9,)),
            pltpu.SemaphoreType.DMA(()),
        ],
        compiler_params=pltpu.CompilerParams(vmem_limit_bytes=100 * 1024 * 1024),
    )(A_x.reshape(S, D).T, A_wqkv, A_wo, B_w1, B_b1, B_w2, B_b2)
    return out.T.reshape(1, S, D)
```
